```python
import os as _os
_os.environ.setdefault("JAX_PLATFORMS", "cpu")
import jax
import jax.numpy as jnp

def _softmax(x, axis=-1):
    return jax.nn.softmax(x, axis=axis)
def _gelu(x):
    return jax.nn.gelu(x, approximate=True)
def _silu(x):
    return jax.nn.silu(x)
def _sigmoid(x):
    return jax.nn.sigmoid(x)
def _layernorm(x, axis=-1, eps=1e-5):
    m = jnp.mean(x, axis=axis, keepdims=True)
    v = jnp.var(x, axis=axis, keepdims=True)
    return (x - m) / jnp.sqrt(v + eps)
def _scatter_add(tgt, idx, src, axis=0):
    return tgt.at[idx].add(src)
def _segment_sum(src, seg, n):
    return jax.ops.segment_sum(src, seg, n)
class _Rng:
    def __init__(self, key):
        self._k = key
    def _next(self):
        self._k, sub = jax.random.split(self._k)
        return sub
    def normal(self, shape):
        return jax.random.normal(self._next(), shape, dtype=jnp.bfloat16)
    def randint(self, lo, hi, shape):
        return jax.random.randint(self._next(), shape, lo, hi, dtype=jnp.int32)
    def uniform(self, shape, lo=0.0, hi=1.0):
        return jax.random.uniform(self._next(), shape, jnp.bfloat16, lo, hi)
    def permutation(self, n):
        return jax.random.permutation(self._next(), n)


kernel_name = 'sequential_preLN__ssm_conv_h3__mixer_s_mlp__prompt'

def setup_inputs():
    _rng = _Rng(jax.random.key(int.from_bytes(__import__("os").urandom(4), "little")))
    _w = (lambda a: (lambda t: t.astype(jnp.bfloat16) if jnp.issubdtype(t.dtype, jnp.floating) else t)(jnp.asarray(a)))
    def _A_setup():
        B, S, D = 1, 2048, 640
        ks = 4
        return {
            "q": _w((lambda *s: _rng.normal(s) * 0.05)(B, S, D)),
            "k": _w((lambda *s: _rng.normal(s) * 0.05)(B, S, D)),
            "v": _w((lambda *s: _rng.normal(s) * 0.05)(B, S, D)),
            "shift_k": _w((lambda *s: _rng.normal(s) * 0.05)(D, ks) * 0.5),
            "ssm_k": _w((lambda *s: _rng.normal(s) * 0.05)(D, S) * (1.0 / S ** 0.5)),
            "ssm_D": _w((lambda *s: _rng.normal(s) * 0.05)(D)),
        }
    _A_in = _A_setup()

    def _B_setup():
        B, S, D, F = 1, 2048, 640, 1728
        return {
            "x":  _w((lambda *s: _rng.normal(s) * 0.05)(B, S, D)),
            "w1": _w((lambda *s: _rng.normal(s) * 0.8)(D, D) * (D ** -0.5)),
            "w2": _w((lambda *s: _rng.normal(s) * 0.8)(D, D) * (D ** -0.5)),
            "w3": _w((lambda *s: _rng.normal(s) * 0.8)(D, F) * (D ** -0.5)),
            "w4": _w((lambda *s: _rng.normal(s) * 0.8)(F, D) * (F ** -0.5)),
        }
    _B_in = _B_setup()

    return {
        "A_q": _A_in["q"],
        "A_k": _A_in["k"],
        "A_v": _A_in["v"],
        "A_shift_k": _A_in["shift_k"],
        "A_ssm_k": _A_in["ssm_k"],
        "A_ssm_D": _A_in["ssm_D"],
        "B_x": _B_in["x"],
        "B_w1": _B_in["w1"],
        "B_w2": _B_in["w2"],
        "B_w3": _B_in["w3"],
        "B_w4": _B_in["w4"],
    }

def reference(A_q, A_k, A_v, A_shift_k, A_ssm_k, A_ssm_D, B_x, B_w1, B_w2, B_w3, B_w4):
    def _A_ref(q, k, v, shift_k, ssm_k, ssm_D):
        B, S, D = q.shape
        ks = shift_k.shape[-1]
        k_pad = jnp.pad(k, ((0, 0), (ks - 1, 0), (0, 0)))
        k_shift = jnp.zeros_like(k)
        for t in range(ks):
            k_shift = k_shift + k_pad[:, t:t + S, :] * shift_k[:, ks - 1 - t][None, None, :]
        kv = k_shift * v
        L = 2 * S
        kv_pad = jnp.pad(kv, ((0, 0), (0, S), (0, 0)))
        kf_pad = jnp.pad(ssm_k, ((0, 0), (0, S)))
        kv_f = (lambda x, axes=(-2,-1): jnp.fft.rfft2(x.astype(jnp.float32), axes=axes))(kv_pad[:, None, :, :], axes=(1, 2))
        kf_f = (lambda x, axes=(-2,-1): jnp.fft.rfft2(x.astype(jnp.float32), axes=axes))(kf_pad[:, None, :], axes=(1, 2))
        kf_f = (lambda x, *d: x.transpose(*d))(kf_f, 1, 2, 0)
        y_f = kv_f * kf_f[None, :, :, :]
        y = (lambda x, s, axes=(-2,-1): jnp.fft.irfft2(x, s=s, axes=axes).astype(jnp.bfloat16))(y_f, (1, L), axes=(1, 2))[:, 0, :S, :]
        y = y + kv * ssm_D[None, None, :]
        return q * y

    def _B_ref(x, w1, w2, w3, w4):
        B, S, D = x.shape
        h = _gelu(_layernorm(x, axis=-1) @ w1)
        c = D // 4
        g0 = jnp.pad(h[:, :, 0*c:1*c], ((0, 0), (1, 0), (0, 0)))[:, :S, :]
        g1 = jnp.pad(h[:, :, 1*c:2*c], ((0, 0), (0, 1), (0, 0)))[:, 1:, :]
        g2 = jnp.pad(h[:, :, 2*c:3*c], ((0, 0), (2, 0), (0, 0)))[:, :S, :]
        g3 = jnp.pad(h[:, :, 3*c:   ], ((0, 0), (0, 2), (0, 0)))[:, 2:, :]
        hs = jnp.concatenate([g0, g1, g2, g3], axis=-1) @ w2
        x1 = x + hs
        h2 = _gelu(_layernorm(x1, axis=-1) @ w3) @ w4
        return x1 + h2

    x = A_q
    h = x + _A_ref(_layernorm(x, axis=-1), A_k, A_v, A_shift_k, A_ssm_k, A_ssm_D)
    h2 = h + _B_ref(_layernorm(h, axis=-1), B_w1, B_w2, B_w3, B_w4)
    return h2
```

```python
import collections
import numpy as np
import jax
import jax.numpy as jnp
from jax.experimental import pallas as pl
from jax.experimental.pallas import tpu as pltpu

S, D, F, KS = 2048, 640, 1728, 4
C = 128
NC = S // C
T = D // 128
NF = -(-F // 128)
EPS = 1e-5
f32, bf16, u32 = jnp.float32, jnp.bfloat16, jnp.uint32


def dft_consts():
    n = np.arange(C)[None, :]
    k = np.concatenate([np.arange(0, C, 2), np.arange(1, C, 2)])[:, None]
    th = 2 * np.pi * n * (k + 0.5) / (2 * C)
    fr, fi = np.cos(th), -np.sin(th)
    Ff = np.concatenate([np.concatenate([fr[16 * j:16 * j + 16], fi[16 * j:16 * j + 16]], 0) for j in range(8)], 0)
    G = Ff.T / C
    return Ff.astype(np.float32), G.astype(np.float32)


GC = float(np.sqrt(2.0 / np.pi))


class Sched:
    def __init__(self, rho, dry, cap=150.0, rrw=4000.0, verbose=False):
        self.cap = cap
        self.rrw = rrw
        self.t = 0.0
        self.rho = rho
        self.dry = dry
        self.ev = {}
        self.groups = []
        self.tasks = []
        self.credit = 0.0
        self.idle = 0.0
        self.verbose = verbose
        self.dma_wait = {}
        self.dma_time = {}
        self.waited = set()
        self.log = []
        self.rr = 0

    def add_group(self, name, key, deps, pieces, post_cost, emit, dma=None):
        self.groups.append(dict(name=name, key=key, deps=deps, pieces=pieces, post=post_cost, emit=emit, dma=dma))

    def add_task(self, name, deadline, deps, gen, dma=None):
        self.tasks.append(dict(name=name, dl=deadline, deps=deps, gen=gen(), ok=0.0, dma=dma, started=False))

    def ready_time(self, x):
        tr = 0.0
        for e, lat in x["deps"]:
            if e not in self.ev:
                return None
            tr = max(tr, self.ev[e] + lat)
        if x["dma"] is not None:
            tr = max(tr, self.dma_time[x["dma"]])
        return tr

    def need_dma(self, x):
        g = x["dma"]
        if g is not None and g not in self.waited:
            self.waited.add(g)
            self.log.append((self.t, "WAIT %s" % g))
            if not self.dry:
                self.dma_wait[g]()
            self.t += 200
            self.credit = 0

    def step_task(self, tk):
        if not tk["started"]:
            self.need_dma(tk)
            tk["started"] = True
        try:
            r = next(tk["gen"])
            cost, gap = r if isinstance(r, tuple) else (r, 0)
            tk["ok"] = self.t + gap
            return cost
        except StopIteration:
            self.ev[tk["name"]] = self.t
            self.tasks.remove(tk)
            return 0

    def eligible(self, slack=0.0):
        out = []
        for tk in self.tasks:
            tr = tk.get("rt")
            if tr is None:
                tr = self.ready_time(tk)
                if tr is None:
                    continue
                tk["rt"] = tr
            if tr <= self.t + slack and tk["ok"] <= self.t + slack:
                out.append(tk)
        out.sort(key=lambda x: x["dl"])
        return out

    def fill(self):
        while self.credit > 0:
            el = self.eligible()
            if not el:
                break
            self.rr += 1
            tk = el[self.rr % 2] if len(el) > 1 and el[1]["dl"] <= el[0]["dl"] + self.rrw else el[0]
            self.credit -= self.step_task(tk)

    def run(self):
        while self.groups:
            best, bt = None, None
            soon, st = None, None
            for g in self.groups:
                tr = self.ready_time(g)
                if tr is None:
                    continue
                if tr <= self.t:
                    if best is None or g["key"] < best["key"]:
                        best = g
                elif soon is None or tr < st:
                    soon, st = g, tr
            if best is None:
                el = self.eligible()
                if el:
                    c = self.step_task(el[0])
                    dt = c / 3.6
                    self.t += dt
                    self.idle += dt
                    self.credit = 0
                    continue
                nt = [st] if soon is not None else []
                for tk in self.tasks:
                    tr = tk.get("rt") or self.ready_time(tk)
                    if tr is not None:
                        nt.append(max(tr, tk["ok"]))
                assert nt, ("deadlock", [g["name"] for g in self.groups][:10], [t["name"] for t in self.tasks][:10])
                nt = min(x for x in nt)
                self.idle += max(nt - self.t, 0)
                self.t = max(nt, self.t + 1e-3)
                continue
            self.need_dma(best)
            self.groups.remove(best)
            self.log.append((self.t, str(best["name"])))
            gen = best["emit"]()
            npc = len(best["pieces"])
            for i, c in enumerate(best["pieces"]):
                next(gen)
                self.t += c
                self.credit += c * 4 * self.rho
                if i == npc - 1:
                    self.credit -= best["post"]
                    self.ev[best["name"]] = self.t
                self.credit = min(self.credit, self.cap)
                self.fill()
            for _ in gen:
                pass
        while self.tasks:
            el = self.eligible(slack=1e9)
            assert el
            c = self.step_task(el[0])
            self.t += c / 3.6
        return self


def build(sc, R, P):
    dry = sc.dry
    CP = 7040.0
    LA, LB = P["LA"], P["LB"]
    st = {}

    def ld8(ref, idx, r0, n):
        parts = [ref[idx + (pl.ds(r0 + 8 * i, 8), slice(None))].astype(f32) for i in range(n // 8)]
        return parts[0] if len(parts) == 1 else jnp.concatenate(parts, axis=0)

    def pack_store(ref, idx, r0, val):
        n = val.shape[0]
        ref[idx + (pl.ds(r0, n), slice(None))] = val.astype(bf16)

    def ldp(ref, idx, r0, n):
        return pltpu.bitcast(ref.bitcast(u32)[idx + (pl.ds(r0 // 2, n // 2), slice(None))], bf16)

    def mm(a, b):
        return jnp.dot(a, b, preferred_element_type=f32)

    def mm_nt(a, b):
        return jax.lax.dot_general(a, b, (((1,), (1,)), ((), ())), preferred_element_type=f32)

    def gelu_x2(x):
        u = x * x
        u = u * (0.044715 * GC) + GC
        return x * jnp.tanh(u * x) + x

    def gelu2(x):
        u = x * x
        u = u * (0.044715 * GC) + GC
        t = jnp.tanh(u * x)
        hx = 0.5 * x
        return hx * t + hx

    def coef_gen():
        if not dry:
            sk = R.sk_in[...].astype(f32)
            for t in range(T):
                for j in range(KS):
                    R.skb[j, t] = jnp.broadcast_to(sk[j:j + 1, t * 128:(t + 1) * 128], (8, 128))
            dd = R.d_in[...].astype(f32)
            for t in range(T):
                R.db[t] = jnp.broadcast_to(dd[t:t + 1, :], (8, 128))
            z = jnp.zeros((8, 128), f32)
            for t in range(T):
                R.kf[t, pl.ds(0, 8), :] = z
                R.hh[t, pl.ds(0, 8), :] = z
                R.hh[t, pl.ds(8 + S, 8), :] = z
        yield 60
    sc.add_task(("coef",), -20, [], coef_gen, dma=P["dma_c"])

    def kv_task(a, t):
        def gen():
            for r0 in range(0, C, 32):
                if not dry:
                    R.kf[t, pl.ds(8 + a * C + r0, 32), :] = ld8(R.k_in, (t,), a * C + r0, 32)
                yield 4
            if not dry:
                cf = [R.skb[j, t] for j in range(KS)]
            for r0 in range(0, C, 16):
                if not dry:
                    outs = []
                    for i in range(2):
                        b = 8 + a * C + r0 + 8 * i
                        acc = R.kf[t, pl.ds(b, 8), :] * cf[0]
                        for j in range(1, KS):
                            acc = acc + R.kf[t, pl.ds(b - j, 8), :] * cf[j]
                        outs.append(acc * R.v_in[t, pl.ds(a * C + r0 + 8 * i, 8), :].astype(f32))
                    pack_store(R.kv, (a, t), r0, jnp.concatenate(outs, axis=0))
                yield 19
        deps = [(("coef",), 0)] + ([(("kv", a - 1, t), 0)] if a > 0 else [])
        sc.add_task(("kv", a, t), (a - LA) * CP + t * P["aS"] + P["aO"] - 600, deps, gen, dma=P["dma_x"][a])

    def au_group(a, t):
        def emit():
            if not dry:
                d = mm(ldp(R.ff_in, (0,), 0, 256), ldp(R.kv, (a, t), 0, C))
                for j in range(8):
                    ur = d[32 * j:32 * j + 16]
                    ui = d[32 * j + 16:32 * j + 32]
                    R.u[a, 0, t, pl.ds(16 * j, 16), :] = ur
                    R.u[a, 1, t, pl.ds(16 * j, 16), :] = ui
                    R.u[a, 2, t, pl.ds(16 * j, 16), :] = ur + ui
            yield
        sc.add_group(("AU", a, t), (a - LA) * CP + t * P["aS"] + P["aO"], [(("kv", a, t), 200)], [64], 16, emit, dma=P["dma_c"])

    def ak_group(a, t):
        def emit():
            if not dry:
                d = mm_nt(ldp(R.ff_in, (0,), 0, 256), ldp(R.sk_s, (a,), 128 * t, 128))
                for j in range(8):
                    kr = d[32 * j:32 * j + 16]
                    ki = d[32 * j + 16:32 * j + 32]
                    rows = pl.ds(16 * j, 16)
                    if a == 0:
                        dv = R.db[t]
                        kr = kr + jnp.concatenate([dv, dv], axis=0)
                        tr, ti = kr, ki
                    else:
                        pr = R.kh[(a - 1) % 2, 0, t, rows, :]
                        pi = R.kh[(a - 1) % 2, 1, t, rows, :]
                        if j < 4:
                            tr, ti = kr - pi, ki + pr
                        else:
                            tr, ti = kr + pi, ki - pr
                    if a < NC - 1:
                        R.kh[a % 2, 0, t, rows, :] = kr
                        R.kh[a % 2, 1, t, rows, :] = ki
                    R.kt[a, 0, t, rows, :] = tr
                    R.kt[a, 1, t, rows, :] = ti - tr
                    R.kt[a, 2, t, rows, :] = tr + ti
            yield
        deps = [(("coef",), 0)] + ([(("AK", a - 1, t), 260)] if a > 0 else [])
        sc.add_group(("AK", a, t), (a - LA) * CP + t * P["aS"] + P["aO"] + 64, deps, [64], 64, emit, dma=P["dma_x"][a])

    def pw_task(s, t):
        a = 2 * s
        def gen():
            PWR = P["PWR"]
            hold = {}
            for j in range(C // PWR):
                rows = pl.ds(PWR * j, PWR)
                if not dry:
                    acc = [[None] * 3, [None] * 3]

                    def add(o, p, v):
                        acc[o][p] = v if acc[o][p] is None else acc[o][p] + v
                    uc = {}

                    def U(n_):
                        if n_ not in uc:
                            uc[n_] = [R.u[n_, p, t, rows, :] for p in range(3)]
                        return uc[n_]
                if P["mid"]:
                    order = sorted(range(a + 2), key=lambda m_: (max(m_, a + 1 - m_), m_))
                else:
                    order = list(range(a + 2))
                for i_, m in enumerate(order):
                    if not dry:
                        kk = [R.kt[m, p, t, rows, :] for p in range(3)]
                        for o in (1, 0):
                            if m > a + o:
                                continue
                            u = U(a + o - m)
                            add(o, 0, kk[0] * u[2])
                            add(o, 1, kk[1] * u[0])
                            add(o, 2, kk[2] * u[1])
                    yield ((24 if i_ > 0 else 12) if m <= a else 12) * PWR // 16
                if not dry:
                    for o in range(2):
                        zr = acc[o][0] - acc[o][2]
                        zi = acc[o][0] + acc[o][1]
                        if PWR == 8:
                            if j % 2 == 0:
                                hold[o] = (zr, zi)
                                continue
                            zr = jnp.concatenate([hold[o][0], zr], axis=0)
                            zi = jnp.concatenate([hold[o][1], zi], axis=0)
                        jj = (PWR * j) // 16
                        pack_store(R.zz, ((a + o) % P["ZS"], t), 32 * jj, zr)
                        pack_store(R.zz, ((a + o) % P["ZS"], t), 32 * jj + 16, zi)
                yield 12 * PWR // 16
        deps = [(("AU", a + 1, t), 260), (("AK", a + 1, t), 260), (("AU", a, t), 260)]
        if a + 1 >= P["ZS"]:
            deps += [(("B", a + 1 - P["ZS"], t), 0)]
        sc.add_task(("pw", s, t), (a - LB - 0.05) * CP + t, deps, gen)

    def rsq(v):
        if P["fastr"]:
            return jnp.exp2(jnp.log2(v) * -0.5)
        return jax.lax.rsqrt(v)

    def ln_steps(load, both=False):
        if not dry:
            xs = load()
            s_ = xs[0] + xs[1] + xs[2] + xs[3] + xs[4]
            m = jnp.sum(s_, axis=-1, keepdims=True) * (1.0 / D)
        yield (12, P["lng"])
        if not dry:
            xc = [x - m for x in xs]
            q_ = xc[0] * xc[0]
            for x in xc[1:]:
                q_ = q_ + x * x
            v = jnp.sum(q_, axis=-1, keepdims=True) * (1.0 / D) + EPS
        yield (32, P["lng"])
        if not dry:
            r = rsq(v)
            o = [x * r for x in xc]
            if both:
                r2 = rsq((v - EPS) * (r * r) + EPS)
                o = (o, [x * r2 for x in o])
        else:
            o = None
        yield (14 + (20 if both else 0), 0)
        return o

    def lnx_task(a):
        def gen():
            for r0 in range(0, C, 16):
                def load():
                    xs = [ld8(R.q_in, (t,), a * C + r0, 16) for t in range(T)]
                    for t in range(T):
                        R.xf[a % P["XS"], t, pl.ds(r0, 16), :] = xs[t]
                    return xs
                o = yield from ln_steps(load)
                if not dry:
                    for t in range(T):
                        R.qn[a % P["XS"], t, pl.ds(r0, 16), :] = o[t]
                yield 10
        deps = [(("B", a - P["XS"], t), 0) for t in range(T)] if a >= P["XS"] else []
        sc.add_task(("lnx", a), (a - LB - 0.3) * CP, deps, gen, dma=P["dma_x"][a])

    def b_group(a, t):
        def emit():
            if not dry:
                d0 = mm(ldp(R.g_in, (0,), 0, 128), ldp(R.zz, (a % P["ZS"], t), 0, 128))
            yield
            if not dry:
                d1 = mm(ldp(R.g_in, (1,), 0, 128), ldp(R.zz, (a % P["ZS"], t), 128, 128))
                y = d0 + d1
                sl = a % P["XS"]
                R.h[t, pl.ds(a * C, C), :] = R.xf[sl, t] + R.qn[sl, t] * y
            yield
        sc.add_group(("B", a, t), (a - LB) * CP + t * 64, [(("pw", a // 2, t), 200), (("lnx", a), 0)], [32, 32], 48, emit)

    def lnh_task(a):
        def gen():
            for r0 in range(0, C, 16):
                rows = pl.ds(a * C + r0, 16)
                o = yield from ln_steps(lambda: [R.h[t, rows, :] for t in range(T)], True)
                if not dry:
                    zs, o = o
                    for t in range(T):
                        R.z[t, rows, :] = zs[t]
                    for t in range(T):
                        pack_store(R.z2, (a % P["RS"], t), r0, o[t])
                yield 5
        deps = [(("B", a, t), 260) for t in range(T)]
        if a >= P["RS"]:
            deps += [(("C", a - P["RS"], n), 0) for n in range(T)]
        sc.add_task(("lnh", a), (a - LB) * CP + P["oC"] - 300, deps, gen)

    def c_group(a, n):
        def emit():
            acc = None
            for k in range(T):
                if not dry:
                    d = mm(ldp(R.z2, (a % P["RS"], k), 0, C), ldp(R.w1_in, (n,), 128 * k, 128))
                    acc = d if acc is None else acc + d
                    if k == T - 1:
                        R.hh[n, pl.ds(8 + a * C, C), :] = gelu2(acc)
                yield
        sc.add_group(("C", a, n), (a - LB) * CP + P["oC"] + n * 160, [(("lnh", a), 96)], [32] * T, 64 + 112, emit, dma=P["dma_w1"])

    def hs_task(a, t):
        def gen():
            cfg = {0: (128, -1, -1), 1: (32, -1, 1), 2: (64, 1, -2), 3: (96, -2, 2), 4: (0, 2, 2)}[t]
            split, s0, s1 = cfg
            for r0 in range(0, C, 32):
                if not dry:
                    b = 8 + a * C + r0
                    if split == 128:
                        val = R.hh[t, pl.ds(b + s0, 32), :]
                    elif split == 0:
                        val = R.hh[t, pl.ds(b + s1, 32), :]
                    else:
                        lane = jax.lax.broadcasted_iota(jnp.int32, (32, 128), 1)
                        val = jnp.where(lane < split, R.hh[t, pl.ds(b + s0, 32), :], R.hh[t, pl.ds(b + s1, 32), :])
                    pack_store(R.hs, (a % P["RS"], t), r0, val)
                yield 2 + (4 if 0 < split < 128 else 0)
        deps = [(("C", a, t), 260)]
        if a + 1 < NC:
            deps.append((("C", a + 1, t), 260))
        if a >= P["RS"]:
            deps += [(("D", a - P["RS"], n), 0) for n in range(T)]
        sc.add_task(("hs", a, t), (a + 1) * CP + P["oD"] - 300 + t, deps, gen)

    def d_group(a, n):
        def emit():
            acc = None
            for k in range(T):
                if not dry:
                    d = mm(ldp(R.hs, (a % P["RS"], k), 0, C), ldp(R.w2_in, (n,), 128 * k, 128))
                    acc = d if acc is None else acc + d
                    if k == T - 1:
                        rows = pl.ds(a * C, C)
                        R.x1[n, rows, :] = R.z[n, rows, :] + acc
                yield
        sc.add_group(("D", a, n), (a + 1) * CP + P["oD"] + n * 160, [(("hs", a, t), 96) for t in range(T)], [32] * T, 80, emit, dma=P["dma_w2"])

    def lnx1_task(a):
        def gen():
            for r0 in range(0, C, 16):
                rows = pl.ds(a * C + r0, 16)
                o = yield from ln_steps(lambda: [R.x1[t, rows, :] for t in range(T)])
                if not dry:
                    for t in range(T):
                        pack_store(R.x1n, (a, t), r0, o[t])
                yield 5
        sc.add_task(("lnx1", a), (a + 2) * CP + P["oE"] - 1500, [(("D", a, n), 260) for n in range(T)], gen)

    def e_group(a, n):
        w = min(128, F - 128 * n)
        def emit():
            acc = None
            for k in range(T):
                if not dry:
                    d = mm_nt(ldp(R.x1n, (a, k), 0, C), ldp(R.w3_in, (k,), 128 * n, w))
                    acc = d if acc is None else acc + d
                    if k == T - 1:
                        val = gelu_x2(acc).astype(bf16)
                        if w == 128:
                            R.y3[a % P["YS"], n] = val
                        else:
                            R.y3[a % P["YS"], n, :, pl.ds(0, w)] = val
                yield
        deps = [(("lnx1", a), 96)]
        if a >= P["YS"]:
            deps += [(("F", a - P["YS"], m), 0) for m in range(T)]
        sc.add_group(("E", a, n), (a + 2) * CP + P["oE"] + n * 170, deps, [32] * T, 64 + 96 + 8, emit, dma=P["dma_w3"])

    def f_group(a, n):
        def emit():
            acc = None
            for k in range(NF):
                w = min(128, F - 128 * k)
                if not dry:
                    if w == 128:
                        lhs = ldp(R.y3, (a % P["YS"], k), 0, C)
                    else:
                        lhs = R.y3[a % P["YS"], k, :, pl.ds(0, w)]
                    d = mm(lhs, ldp(R.w4_in, (n,), 128 * k, w))
                    acc = d if acc is None else acc + d
                    if k == NF - 1:
                        rows = pl.ds(a * C, C)
                        R.out[n, rows, :] = (R.h[n, rows, :] + (R.x1[n, rows, :] + acc * 0.5)).astype(bf16)
                        cp = pltpu.make_async_copy(R.out.at[n, rows, :], R.o_hbm.at[rows, pl.ds(128 * n, 128)], R.osem.at[0])
                        cp.start()
                        st.setdefault("outs", []).append(cp)
                yield
        deps = [(("E", a, m), 300) for m in range(NF)]
        sc.add_group(("F", a, n), (a + 3) * CP + P["oF"] + n * 448 + (800 if n >= P["fsplit"] else 0) + (800 if n >= P["fsplit2"] else 0), deps, [32] * NF, 13 * 16 + 56, emit, dma=P["dma_w4"])

    for a in range(NC):
        for t in range(T):
            kv_task(a, t)
            au_group(a, t)
            ak_group(a, t)
            b_group(a, t)
            c_group(a, t)
            hs_task(a, t)
            d_group(a, t)
            f_group(a, t)
            if a % 2 == 0:
                pw_task(a // 2, t)
        lnx_task(a)
        lnh_task(a)
        lnx1_task(a)
        for n in range(NF):
            e_group(a, n)
    return st


DEFAULTS = dict(mid=1, PWR=16, fastr=1, LA=3.0, LB=0.0, aS=1400.0, aO=300.0, oC=1800.0, oD=3500.0, oE=4300.0, oF=350.0, fsplit=3, fsplit2=9, rr=4000.0, lng=60.0, cap=150.0, rho=0.5, ZS=4, XS=4, RS=3, YS=2,
                dma_groups="0-1|w1,2-3|w2,4-5|w3,6-7|w4,8-9|10-15",
                dma_times="2500,8000,12000,19000,26000,34000")


def params(**kw):
    P = dict(DEFAULTS)
    for k, v in kw.items():
        P[k] = type(DEFAULTS[k])(v)
    groups = P["dma_groups"].split("|")
    P["dma_x"] = [None] * NC
    P["dma_c"] = 0
    for gi, g in enumerate(groups):
        for tok in g.split(","):
            if tok.startswith("w"):
                P["dma_" + tok] = gi
            else:
                lo, hi = tok.split("-")
                for a in range(int(lo), int(hi) + 1):
                    P["dma_x"][a] = gi
    P["ngroups"] = len(groups)
    P["times"] = [float(x) for x in P["dma_times"].split(",")]
    return P


def make_kernel(P):
    names = ["q_hbm", "k_hbm", "v_hbm", "sk_hbm", "ssmk_hbm", "d_hbm", "w1_hbm", "w2_hbm", "w3t_hbm", "w4_hbm", "ff_hbm", "g_hbm",
             "o_hbm",
             "q_in", "k_in", "v_in", "sk_in", "sk_s", "d_in", "w1_in", "w2_in", "w3_in", "w4_in", "ff_in", "g_in",
             "skb", "db", "kf", "kv", "u", "kt", "kh", "zz", "xf", "qn",
             "h", "z", "z2", "hh", "hs", "x1", "x1n", "y3", "out", "isem", "osem"]

    def kernel(*refs):
        R = collections.namedtuple("Refs", names)(*refs)
        groups = [[] for _ in range(P["ngroups"])]

        def add(g, src, dst):
            groups[g].append(pltpu.make_async_copy(src, dst, R.isem.at[g]))
        add(P["dma_c"], R.ff_hbm, R.ff_in.at[0])
        add(P["dma_c"], R.g_hbm.at[:, pl.ds(0, 128)], R.g_in.at[0])
        add(P["dma_c"], R.g_hbm.at[:, pl.ds(128, 128)], R.g_in.at[1])
        add(P["dma_c"], R.sk_hbm, R.sk_in)
        add(P["dma_c"], R.d_hbm, R.d_in)
        byg = {}
        for a in range(NC):
            byg.setdefault(P["dma_x"][a], []).append(a)
        for g, lst in byg.items():
            lo, n = lst[0] * C, len(lst) * C
            for a in lst:
                add(g, R.ssmk_hbm.at[:, pl.ds(a * C, C)], R.sk_s.at[a])
            for t in range(T):
                for src, dst in ((R.k_hbm, R.k_in), (R.v_hbm, R.v_in), (R.q_hbm, R.q_in)):
                    add(g, src.at[pl.ds(lo, n), pl.ds(128 * t, 128)], dst.at[t, pl.ds(lo, n), :])
        for nm, src, dst in (("w1", R.w1_hbm, R.w1_in), ("w2", R.w2_hbm, R.w2_in), ("w3", R.w3t_hbm, R.w3_in), ("w4", R.w4_hbm, R.w4_in)):
            for t in range(T):
                add(P["dma_" + nm], src.at[:, pl.ds(128 * t, 128)], dst.at[t])

        sc = Sched(P["rho"], dry=False, cap=P["cap"], rrw=P["rr"])
        started = [0]

        def start_upto(g):
            while started[0] <= min(g, len(groups) - 1):
                for c in groups[started[0]]:
                    c.start()
                started[0] += 1
        start_upto(1)

        def mkwait(g):
            def w():
                for gg in range(g + 1):
                    if gg not in done:
                        start_upto(gg)
                        for c in groups[gg]:
                            c.wait()
                        done.add(gg)
                start_upto(g + 2)
            return w
        done = set()
        for g in range(len(groups)):
            sc.dma_wait[g] = mkwait(g)
            sc.dma_time[g] = P["times"][g] - P["times"][0]
        orig = sc.need_dma

        def need(x):
            g = x["dma"]
            if g is not None and g not in sc.waited:
                orig(x)
                for gg in range(g):
                    sc.waited.add(gg)
        sc.need_dma = need
        st = build(sc, R, P)
        sc.run()
        for cp in st["outs"]:
            cp.wait()
    return kernel


def get_fn(**kw):
    flags = kw.pop("flags", "")
    fl = {k: True for k in flags.split(",") if k}
    P = params(**kw)
    Ff, G = dft_consts()
    kern = make_kernel(P)
    V = pltpu.VMEM
    scratch = [
        V((T, S, 128), bf16), V((T, S, 128), bf16), V((T, S, 128), bf16),
        V((KS, D), bf16), V((NC, D, 128), bf16), V((T, 128), bf16),
        V((T, D, 128), bf16), V((T, D, 128), bf16), V((T, F, 128), bf16), V((T, F, 128), bf16),
        V((1, 256, 128), bf16), V((2, 128, 128), bf16),
        V((KS, T, 8, 128), f32), V((T, 8, 128), f32),
        V((T, S + 8, 128), f32),
        V((NC, T, 128, 128), bf16),
        V((NC, 3, T, 128, 128), f32), V((NC, 3, T, 128, 128), f32), V((2, 2, T, 128, 128), f32),
        V((P["ZS"], T, 256, 128), bf16),
        V((P["XS"], T, 128, 128), f32), V((P["XS"], T, 128, 128), f32),
        V((T, S, 128), f32), V((T, S, 128), f32),
        V((P["RS"], T, 128, 128), bf16),
        V((T, S + 16, 128), f32),
        V((P["RS"], T, 128, 128), bf16),
        V((T, S, 128), f32),
        V((NC, T, 128, 128), bf16),
        V((P["YS"], NF, 128, 128), bf16),
        V((T, S, 128), bf16),
        pltpu.SemaphoreType.DMA((P["ngroups"],)), pltpu.SemaphoreType.DMA((1,)),
    ]

    def fn(A_q, A_k, A_v, A_shift_k, A_ssm_k, A_ssm_D, B_x, B_w1, B_w2, B_w3, B_w4):
        out = pl.pallas_call(
            kern,
            out_shape=jax.ShapeDtypeStruct((S, D), bf16),
            in_specs=[pl.BlockSpec(memory_space=pl.ANY)] * 12,
            out_specs=pl.BlockSpec(memory_space=pl.ANY),
            scratch_shapes=scratch,
            compiler_params=pltpu.CompilerParams(vmem_limit_bytes=120 * 1024 * 1024, flags=fl or None),
        )(A_q.reshape(S, D), A_k.reshape(S, D), A_v.reshape(S, D), A_shift_k.T, A_ssm_k, A_ssm_D.reshape(T, 128),
          B_w1, B_w2, B_w3.T, B_w4, jnp.asarray(Ff, bf16), jnp.asarray(G, bf16))
        return out.reshape(1, S, D)
    return fn


@jax.jit
def pallas_sequential_preLN__ssm_conv_h3__mixer_s_mlp__prompt_kernel(
    A_q: jax.Array,
    A_k: jax.Array,
    A_v: jax.Array,
    A_shift_k: jax.Array,
    A_ssm_k: jax.Array,
    A_ssm_D: jax.Array,
    B_x: jax.Array,
    B_w1: jax.Array,
    B_w2: jax.Array,
    B_w3: jax.Array,
    B_w4: jax.Array,
):
    return get_fn(rho="0.45")(A_q, A_k, A_v, A_shift_k, A_ssm_k, A_ssm_D, B_x, B_w1, B_w2, B_w3, B_w4)
```

```python
import collections
import numpy as np
import jax
import jax.numpy as jnp
from jax.experimental import pallas as pl
from jax.experimental.pallas import tpu as pltpu

S, D, F, KS = 2048, 640, 1728, 4
C = 128
NC = S // C
T = D // 128
NF = -(-F // 128)
EPS = 1e-5
f32, bf16, u32 = jnp.float32, jnp.bfloat16, jnp.uint32


def dft_consts():
    n = np.arange(C)[None, :]
    k = np.concatenate([np.arange(0, C, 2), np.arange(1, C, 2)])[:, None]
    th = 2 * np.pi * n * (k + 0.5) / (2 * C)
    fr, fi = np.cos(th), -np.sin(th)
    Ff = np.concatenate([np.concatenate([fr[16 * j:16 * j + 16], fi[16 * j:16 * j + 16]], 0) for j in range(8)], 0)
    G = Ff.T / C
    return Ff.astype(np.float32), G.astype(np.float32)


GC = float(np.sqrt(2.0 / np.pi))


class Sched:
    def __init__(self, rho, dry, cap=150.0, rrw=4000.0, verbose=False):
        self.cap = cap
        self.rrw = rrw
        self.t = 0.0
        self.rho = rho
        self.dry = dry
        self.ev = {}
        self.groups = []
        self.tasks = []
        self.credit = 0.0
        self.idle = 0.0
        self.verbose = verbose
        self.dma_wait = {}
        self.dma_time = {}
        self.waited = set()
        self.log = []
        self.rr = 0

    def add_group(self, name, key, deps, pieces, post_cost, emit, dma=None):
        self.groups.append(dict(name=name, key=key, deps=deps, pieces=pieces, post=post_cost, emit=emit, dma=dma))

    def add_task(self, name, deadline, deps, gen, dma=None):
        self.tasks.append(dict(name=name, dl=deadline, deps=deps, gen=gen(), ok=0.0, dma=dma, started=False))

    def ready_time(self, x):
        tr = 0.0
        for e, lat in x["deps"]:
            if e not in self.ev:
                return None
            tr = max(tr, self.ev[e] + lat)
        if x["dma"] is not None:
            tr = max(tr, self.dma_time[x["dma"]])
        return tr

    def need_dma(self, x):
        g = x["dma"]
        if g is not None and g not in self.waited:
            self.waited.add(g)
            self.log.append((self.t, "WAIT %s" % g))
            if not self.dry:
                self.dma_wait[g]()
            self.t += 200
            self.credit = 0

    def step_task(self, tk):
        if not tk["started"]:
            self.need_dma(tk)
            tk["started"] = True
        try:
            r = next(tk["gen"])
            cost, gap = r if isinstance(r, tuple) else (r, 0)
            tk["ok"] = self.t + gap
            return cost
        except StopIteration:
            self.ev[tk["name"]] = self.t
            self.tasks.remove(tk)
            return 0

    def eligible(self, slack=0.0):
        out = []
        for tk in self.tasks:
            tr = tk.get("rt")
            if tr is None:
                tr = self.ready_time(tk)
                if tr is None:
                    continue
                tk["rt"] = tr
            if tr <= self.t + slack and tk["ok"] <= self.t + slack:
                out.append(tk)
        out.sort(key=lambda x: x["dl"])
        return out

    def fill(self):
        while self.credit > 0:
            el = self.eligible()
            if not el:
                break
            self.rr += 1
            tk = el[self.rr % 2] if len(el) > 1 and el[1]["dl"] <= el[0]["dl"] + self.rrw else el[0]
            self.credit -= self.step_task(tk)

    def run(self):
        while self.groups:
            best, bt = None, None
            soon, st = None, None
            for g in self.groups:
                tr = self.ready_time(g)
                if tr is None:
                    continue
                if tr <= self.t:
                    if best is None or g["key"] < best["key"]:
                        best = g
                elif soon is None or tr < st:
                    soon, st = g, tr
            if best is None:
                el = self.eligible()
                if el:
                    c = self.step_task(el[0])
                    dt = c / 3.6
                    self.t += dt
                    self.idle += dt
                    self.credit = 0
                    continue
                nt = [st] if soon is not None else []
                for tk in self.tasks:
                    tr = tk.get("rt") or self.ready_time(tk)
                    if tr is not None:
                        nt.append(max(tr, tk["ok"]))
                assert nt, ("deadlock", [g["name"] for g in self.groups][:10], [t["name"] for t in self.tasks][:10])
                nt = min(x for x in nt)
                self.idle += max(nt - self.t, 0)
                self.t = max(nt, self.t + 1e-3)
                continue
            self.need_dma(best)
            self.groups.remove(best)
            self.log.append((self.t, str(best["name"])))
            gen = best["emit"]()
            npc = len(best["pieces"])
            for i, c in enumerate(best["pieces"]):
                next(gen)
                self.t += c
                self.credit += c * 4 * self.rho
                if i == npc - 1:
                    self.credit -= best["post"]
                    self.ev[best["name"]] = self.t
                self.credit = min(self.credit, self.cap)
                self.fill()
            for _ in gen:
                pass
        while self.tasks:
            el = self.eligible(slack=1e9)
            assert el
            c = self.step_task(el[0])
            self.t += c / 3.6
        return self


def build(sc, R, P):
    dry = sc.dry
    CP = 7040.0
    LA, LB = P["LA"], P["LB"]
    st = {}

    def ld8(ref, idx, r0, n):
        parts = [ref[idx + (pl.ds(r0 + 8 * i, 8), slice(None))].astype(f32) for i in range(n // 8)]
        return parts[0] if len(parts) == 1 else jnp.concatenate(parts, axis=0)

    def pack_store(ref, idx, r0, val):
        n = val.shape[0]
        ref[idx + (pl.ds(r0, n), slice(None))] = val.astype(bf16)

    def ldp(ref, idx, r0, n):
        return pltpu.bitcast(ref.bitcast(u32)[idx + (pl.ds(r0 // 2, n // 2), slice(None))], bf16)

    def mm(a, b):
        return jnp.dot(a, b, preferred_element_type=f32)

    def mm_nt(a, b):
        return jax.lax.dot_general(a, b, (((1,), (1,)), ((), ())), preferred_element_type=f32)

    def gelu_x2(x):
        u = x * x
        u = u * (0.044715 * GC) + GC
        return x * jnp.tanh(u * x) + x

    def gelu2(x):
        u = x * x
        u = u * (0.044715 * GC) + GC
        t = jnp.tanh(u * x)
        hx = 0.5 * x
        return hx * t + hx

    def coef_gen():
        if not dry:
            sk = R.sk_in[...].astype(f32)
            for t in range(T):
                for j in range(KS):
                    R.skb[j, t] = jnp.broadcast_to(sk[j:j + 1, t * 128:(t + 1) * 128], (8, 128))
            dd = R.d_in[...].astype(f32)
            for t in range(T):
                R.db[t] = jnp.broadcast_to(dd[t:t + 1, :], (8, 128))
            z = jnp.zeros((8, 128), f32)
            for t in range(T):
                R.kf[t, pl.ds(0, 8), :] = z
                R.hh[t, pl.ds(0, 8), :] = z
                R.hh[t, pl.ds(8 + S, 8), :] = z
        yield 60
    sc.add_task(("coef",), -20, [], coef_gen, dma=P["dma_c"])

    def kv_task(a, t):
        def gen():
            for r0 in range(0, C, 32):
                if not dry:
                    R.kf[t, pl.ds(8 + a * C + r0, 32), :] = ld8(R.k_in, (t,), a * C + r0, 32)
                yield 4
            if not dry:
                cf = [R.skb[j, t] for j in range(KS)]
            for r0 in range(0, C, 16):
                if not dry:
                    outs = []
                    for i in range(2):
                        b = 8 + a * C + r0 + 8 * i
                        acc = R.kf[t, pl.ds(b, 8), :] * cf[0]
                        for j in range(1, KS):
                            acc = acc + R.kf[t, pl.ds(b - j, 8), :] * cf[j]
                        outs.append(acc * R.v_in[t, pl.ds(a * C + r0 + 8 * i, 8), :].astype(f32))
                    pack_store(R.kv, (a, t), r0, jnp.concatenate(outs, axis=0))
                yield 19
        deps = [(("coef",), 0)] + ([(("kv", a - 1, t), 0)] if a > 0 else [])
        sc.add_task(("kv", a, t), (a - LA) * CP + t * P["aS"] + P["aO"] - 600, deps, gen, dma=P["dma_x"][a])

    def au_group(a, t):
        def emit():
            if not dry:
                d = mm(ldp(R.ff_in, (0,), 0, 256), ldp(R.kv, (a, t), 0, C))
                for j in range(8):
                    ur = d[32 * j:32 * j + 16]
                    ui = d[32 * j + 16:32 * j + 32]
                    R.u[a, 0, t, pl.ds(16 * j, 16), :] = ur
                    R.u[a, 1, t, pl.ds(16 * j, 16), :] = ui
                    R.u[a, 2, t, pl.ds(16 * j, 16), :] = ur + ui
            yield
        sc.add_group(("AU", a, t), (a - LA) * CP + t * P["aS"] + P["aO"], [(("kv", a, t), 200)], [64], 16, emit, dma=P["dma_c"])

    def ak_group(a, t):
        def emit():
            if not dry:
                d = mm_nt(ldp(R.ff_in, (0,), 0, 256), ldp(R.sk_s, (a,), 128 * t, 128))
                for j in range(8):
                    kr = d[32 * j:32 * j + 16]
                    ki = d[32 * j + 16:32 * j + 32]
                    rows = pl.ds(16 * j, 16)
                    if a == 0:
                        dv = R.db[t]
                        kr = kr + jnp.concatenate([dv, dv], axis=0)
                        tr, ti = kr, ki
                    else:
                        pr = R.kh[(a - 1) % 2, 0, t, rows, :]
                        pi = R.kh[(a - 1) % 2, 1, t, rows, :]
                        if j < 4:
                            tr, ti = kr - pi, ki + pr
                        else:
                            tr, ti = kr + pi, ki - pr
                    if a < NC - 1:
                        R.kh[a % 2, 0, t, rows, :] = kr
                        R.kh[a % 2, 1, t, rows, :] = ki
                    R.kt[a, 0, t, rows, :] = tr
                    R.kt[a, 1, t, rows, :] = ti - tr
                    R.kt[a, 2, t, rows, :] = tr + ti
            yield
        deps = [(("coef",), 0)] + ([(("AK", a - 1, t), 260)] if a > 0 else [])
        sc.add_group(("AK", a, t), (a - LA) * CP + t * P["aS"] + P["aO"] + 64, deps, [64], 64, emit, dma=P["dma_x"][a])

    def pw_task(s, t):
        a = 2 * s
        def gen():
            PWR = P["PWR"]
            hold = {}
            for j in range(C // PWR):
                rows = pl.ds(PWR * j, PWR)
                if not dry:
                    acc = [[None] * 3, [None] * 3]

                    def add(o, p, v):
                        acc[o][p] = v if acc[o][p] is None else acc[o][p] + v
                    uc = {}

                    def U(n_):
                        if n_ not in uc:
                            uc[n_] = [R.u[n_, p, t, rows, :] for p in range(3)]
                        return uc[n_]
                if P["mid"]:
                    order = sorted(range(a + 2), key=lambda m_: (max(m_, a + 1 - m_), m_))
                else:
                    order = list(range(a + 2))
                for i_, m in enumerate(order):
                    if not dry:
                        kk = [R.kt[m, p, t, rows, :] for p in range(3)]
                        for o in (1, 0):
                            if m > a + o:
                                continue
                            u = U(a + o - m)
                            add(o, 0, kk[0] * u[2])
                            add(o, 1, kk[1] * u[0])
                            add(o, 2, kk[2] * u[1])
                    yield ((24 if i_ > 0 else 12) if m <= a else 12) * PWR // 16
                if not dry:
                    for o in range(2):
                        zr = acc[o][0] - acc[o][2]
                        zi = acc[o][0] + acc[o][1]
                        if PWR == 8:
                            if j % 2 == 0:
                                hold[o] = (zr, zi)
                                continue
                            zr = jnp.concatenate([hold[o][0], zr], axis=0)
                            zi = jnp.concatenate([hold[o][1], zi], axis=0)
                        jj = (PWR * j) // 16
                        pack_store(R.zz, ((a + o) % P["ZS"], t), 32 * jj, zr)
                        pack_store(R.zz, ((a + o) % P["ZS"], t), 32 * jj + 16, zi)
                yield 12 * PWR // 16
        deps = [(("AU", a + 1, t), 260), (("AK", a + 1, t), 260), (("AU", a, t), 260)]
        if a + 1 >= P["ZS"]:
            deps += [(("B", a + 1 - P["ZS"], t), 0)]
        sc.add_task(("pw", s, t), (a - LB - 0.05) * CP + t, deps, gen)

    def rsq(v):
        if P["fastr"]:
            return jnp.exp2(jnp.log2(v) * -0.5)
        return jax.lax.rsqrt(v)

    def ln_steps(load, both=False):
        if not dry:
            xs = load()
            s_ = xs[0] + xs[1] + xs[2] + xs[3] + xs[4]
            m = jnp.sum(s_, axis=-1, keepdims=True) * (1.0 / D)
        yield (12, P["lng"])
        if not dry:
            xc = [x - m for x in xs]
            q_ = xc[0] * xc[0]
            for x in xc[1:]:
                q_ = q_ + x * x
            v = jnp.sum(q_, axis=-1, keepdims=True) * (1.0 / D) + EPS
        yield (32, P["lng"])
        if not dry:
            r = rsq(v)
            o = [x * r for x in xc]
            if both:
                r2 = rsq((v - EPS) * (r * r) + EPS)
                o = (o, [x * r2 for x in o])
        else:
            o = None
        yield (14 + (20 if both else 0), 0)
        return o

    def lnx_task(a):
        def gen():
            for r0 in range(0, C, 16):
                def load():
                    xs = [ld8(R.q_in, (t,), a * C + r0, 16) for t in range(T)]
                    for t in range(T):
                        R.xf[a % P["XS"], t, pl.ds(r0, 16), :] = xs[t]
                    return xs
                o = yield from ln_steps(load)
                if not dry:
                    for t in range(T):
                        R.qn[a % P["XS"], t, pl.ds(r0, 16), :] = o[t]
                yield 10
        deps = [(("B", a - P["XS"], t), 0) for t in range(T)] if a >= P["XS"] else []
        sc.add_task(("lnx", a), (a - LB - 0.3) * CP, deps, gen, dma=P["dma_x"][a])

    def b_group(a, t):
        def emit():
            if not dry:
                d0 = mm(ldp(R.g_in, (0,), 0, 128), ldp(R.zz, (a % P["ZS"], t), 0, 128))
            yield
            if not dry:
                d1 = mm(ldp(R.g_in, (1,), 0, 128), ldp(R.zz, (a % P["ZS"], t), 128, 128))
                y = d0 + d1
                sl = a % P["XS"]
                R.h[t, pl.ds(a * C, C), :] = R.xf[sl, t] + R.qn[sl, t] * y
            yield
        sc.add_group(("B", a, t), (a - LB) * CP + t * 64, [(("pw", a // 2, t), 200), (("lnx", a), 0)], [32, 32], 48, emit)

    def lnh_task(a):
        def gen():
            for r0 in range(0, C, 16):
                rows = pl.ds(a * C + r0, 16)
                o = yield from ln_steps(lambda: [R.h[t, rows, :] for t in range(T)], True)
                if not dry:
                    zs, o = o
                    for t in range(T):
                        R.z[t, rows, :] = zs[t]
                    for t in range(T):
                        pack_store(R.z2, (a % P["RS"], t), r0, o[t])
                yield 5
        deps = [(("B", a, t), 260) for t in range(T)]
        if a >= P["RS"]:
            deps += [(("C", a - P["RS"], n), 0) for n in range(T)]
        sc.add_task(("lnh", a), (a - LB) * CP + P["oC"] - 300, deps, gen)

    def c_group(a, n):
        def emit():
            acc = None
            for k in range(T):
                if not dry:
                    d = mm(ldp(R.z2, (a % P["RS"], k), 0, C), ldp(R.w1_in, (n,), 128 * k, 128))
                    acc = d if acc is None else acc + d
                    if k == T - 1:
                        R.hh[n, pl.ds(8 + a * C, C), :] = gelu2(acc)
                yield
        sc.add_group(("C", a, n), (a - LB) * CP + P["oC"] + n * 160, [(("lnh", a), 96)], [32] * T, 64 + 112, emit, dma=P["dma_w1"])

    def hs_task(a, t):
        def gen():
            cfg = {0: (128, -1, -1), 1: (32, -1, 1), 2: (64, 1, -2), 3: (96, -2, 2), 4: (0, 2, 2)}[t]
            split, s0, s1 = cfg
            for r0 in range(0, C, 32):
                if not dry:
                    b = 8 + a * C + r0
                    if split == 128:
                        val = R.hh[t, pl.ds(b + s0, 32), :]
                    elif split == 0:
                        val = R.hh[t, pl.ds(b + s1, 32), :]
                    else:
                        lane = jax.lax.broadcasted_iota(jnp.int32, (32, 128), 1)
                        val = jnp.where(lane < split, R.hh[t, pl.ds(b + s0, 32), :], R.hh[t, pl.ds(b + s1, 32), :])
                    pack_store(R.hs, (a % P["RS"], t), r0, val)
                yield 2 + (4 if 0 < split < 128 else 0)
        deps = [(("C", a, t), 260)]
        if a + 1 < NC:
            deps.append((("C", a + 1, t), 260))
        if a >= P["RS"]:
            deps += [(("D", a - P["RS"], n), 0) for n in range(T)]
        sc.add_task(("hs", a, t), (a + 1) * CP + P["oD"] - 300 + t, deps, gen)

    def d_group(a, n):
        def emit():
            acc = None
            for k in range(T):
                if not dry:
                    d = mm(ldp(R.hs, (a % P["RS"], k), 0, C), ldp(R.w2_in, (n,), 128 * k, 128))
                    acc = d if acc is None else acc + d
                    if k == T - 1:
                        rows = pl.ds(a * C, C)
                        R.x1[n, rows, :] = R.z[n, rows, :] + acc
                yield
        sc.add_group(("D", a, n), (a + 1) * CP + P["oD"] + n * 160, [(("hs", a, t), 96) for t in range(T)], [32] * T, 80, emit, dma=P["dma_w2"])

    def lnx1_task(a):
        def gen():
            for r0 in range(0, C, 16):
                rows = pl.ds(a * C + r0, 16)
                o = yield from ln_steps(lambda: [R.x1[t, rows, :] for t in range(T)])
                if not dry:
                    for t in range(T):
                        pack_store(R.x1n, (a, t), r0, o[t])
                yield 5
        sc.add_task(("lnx1", a), (a + 2) * CP + P["oE"] - 1500, [(("D", a, n), 260) for n in range(T)], gen)

    def e_group(a, n):
        w = min(128, F - 128 * n)
        def emit():
            acc = None
            for k in range(T):
                if not dry:
                    d = mm_nt(ldp(R.x1n, (a, k), 0, C), ldp(R.w3_in, (k,), 128 * n, w))
                    acc = d if acc is None else acc + d
                    if k == T - 1:
                        val = gelu_x2(acc).astype(bf16)
                        if w == 128:
                            R.y3[a % P["YS"], n] = val
                        else:
                            R.y3[a % P["YS"], n, :, pl.ds(0, w)] = val
                yield
        deps = [(("lnx1", a), 96)]
        if a >= P["YS"]:
            deps += [(("F", a - P["YS"], m), 0) for m in range(T)]
        sc.add_group(("E", a, n), (a + 2) * CP + P["oE"] + n * 170, deps, [32] * T, 64 + 96 + 8, emit, dma=P["dma_w3"])

    def f_group(a, n):
        def emit():
            acc = None
            for k in range(NF):
                w = min(128, F - 128 * k)
                if not dry:
                    if w == 128:
                        lhs = ldp(R.y3, (a % P["YS"], k), 0, C)
                    else:
                        lhs = R.y3[a % P["YS"], k, :, pl.ds(0, w)]
                    d = mm(lhs, ldp(R.w4_in, (n,), 128 * k, w))
                    acc = d if acc is None else acc + d
                    if k == NF - 1:
                        rows = pl.ds(a * C, C)
                        R.out[n, rows, :] = (R.h[n, rows, :] + (R.x1[n, rows, :] + acc * 0.5)).astype(bf16)
                        cp = pltpu.make_async_copy(R.out.at[n, rows, :], R.o_hbm.at[rows, pl.ds(128 * n, 128)], R.osem.at[0])
                        cp.start()
                        st.setdefault("outs", []).append(cp)
                yield
        deps = [(("E", a, m), 300) for m in range(NF)]
        sc.add_group(("F", a, n), (a + 3) * CP + P["oF"] + n * 448 + (800 if n >= P["fsplit"] else 0) + (800 if n >= P["fsplit2"] else 0), deps, [32] * NF, 13 * 16 + 56, emit, dma=P["dma_w4"])

    for a in range(NC):
        for t in range(T):
            kv_task(a, t)
            au_group(a, t)
            ak_group(a, t)
            b_group(a, t)
            c_group(a, t)
            hs_task(a, t)
            d_group(a, t)
            f_group(a, t)
            if a % 2 == 0:
                pw_task(a // 2, t)
        lnx_task(a)
        lnh_task(a)
        lnx1_task(a)
        for n in range(NF):
            e_group(a, n)
    return st


DEFAULTS = dict(ahead=2, mid=1, PWR=16, fastr=1, LA=3.0, LB=0.0, aS=1400.0, aO=300.0, oC=1800.0, oD=3500.0, oE=4300.0, oF=350.0, fsplit=3, fsplit2=9, rr=4000.0, lng=60.0, cap=150.0, rho=0.5, ZS=4, XS=4, RS=3, YS=2,
                dma_groups="0-1|w1,2-3|w2,4-5|w3,6-7|w4,8-9|10-15",
                dma_times="2500,8000,12000,19000,26000,34000")


def params(**kw):
    P = dict(DEFAULTS)
    for k, v in kw.items():
        P[k] = type(DEFAULTS[k])(v)
    groups = P["dma_groups"].split("|")
    P["dma_x"] = [None] * NC
    P["dma_c"] = 0
    for gi, g in enumerate(groups):
        for tok in g.split(","):
            if tok.startswith("w"):
                P["dma_" + tok] = gi
            else:
                lo, hi = tok.split("-")
                for a in range(int(lo), int(hi) + 1):
                    P["dma_x"][a] = gi
    P["ngroups"] = len(groups)
    P["times"] = [float(x) for x in P["dma_times"].split(",")]
    return P


def make_kernel(P):
    names = ["q_hbm", "k_hbm", "v_hbm", "sk_hbm", "ssmk_hbm", "d_hbm", "w1_hbm", "w2_hbm", "w3t_hbm", "w4_hbm", "ff_hbm", "g_hbm",
             "o_hbm",
             "q_in", "k_in", "v_in", "sk_in", "sk_s", "d_in", "w1_in", "w2_in", "w3_in", "w4_in", "ff_in", "g_in",
             "skb", "db", "kf", "kv", "u", "kt", "kh", "zz", "xf", "qn",
             "h", "z", "z2", "hh", "hs", "x1", "x1n", "y3", "out", "isem", "osem"]

    def kernel(*refs):
        R = collections.namedtuple("Refs", names)(*refs)
        groups = [[] for _ in range(P["ngroups"])]

        def add(g, src, dst):
            groups[g].append(pltpu.make_async_copy(src, dst, R.isem.at[g]))
        add(P["dma_c"], R.ff_hbm, R.ff_in.at[0])
        add(P["dma_c"], R.g_hbm.at[:, pl.ds(0, 128)], R.g_in.at[0])
        add(P["dma_c"], R.g_hbm.at[:, pl.ds(128, 128)], R.g_in.at[1])
        add(P["dma_c"], R.sk_hbm, R.sk_in)
        add(P["dma_c"], R.d_hbm, R.d_in)
        byg = {}
        for a in range(NC):
            byg.setdefault(P["dma_x"][a], []).append(a)
        for g, lst in byg.items():
            lo, n = lst[0] * C, len(lst) * C
            for a in lst:
                add(g, R.ssmk_hbm.at[:, pl.ds(a * C, C)], R.sk_s.at[a])
            for t in range(T):
                for src, dst in ((R.k_hbm, R.k_in), (R.v_hbm, R.v_in), (R.q_hbm, R.q_in)):
                    add(g, src.at[pl.ds(lo, n), pl.ds(128 * t, 128)], dst.at[t, pl.ds(lo, n), :])
        for nm, src, dst in (("w1", R.w1_hbm, R.w1_in), ("w2", R.w2_hbm, R.w2_in), ("w3", R.w3t_hbm, R.w3_in), ("w4", R.w4_hbm, R.w4_in)):
            for t in range(T):
                add(P["dma_" + nm], src.at[:, pl.ds(128 * t, 128)], dst.at[t])

        sc = Sched(P["rho"], dry=False, cap=P["cap"], rrw=P["rr"])
        started = [0]

        def start_upto(g):
            while started[0] <= min(g, len(groups) - 1):
                for c in groups[started[0]]:
                    c.start()
                started[0] += 1
        start_upto(P["ahead"] - 1)

        def mkwait(g):
            def w():
                for gg in range(g + 1):
                    if gg not in done:
                        start_upto(gg)
                        with jax.named_scope("wait%d" % gg):
                            for c in groups[gg]:
                                c.wait()
                        done.add(gg)
                start_upto(g + P["ahead"])
            return w
        done = set()
        for g in range(len(groups)):
            sc.dma_wait[g] = mkwait(g)
            sc.dma_time[g] = P["times"][g] - P["times"][0]
        orig = sc.need_dma

        def need(x):
            g = x["dma"]
            if g is not None and g not in sc.waited:
                orig(x)
                for gg in range(g):
                    sc.waited.add(gg)
        sc.need_dma = need
        st = build(sc, R, P)
        sc.run()
        with jax.named_scope("waitout"):
            for cp in st["outs"]:
                cp.wait()
    return kernel


def get_fn(**kw):
    flags = kw.pop("flags", "")
    fl = {k: True for k in flags.split(",") if k}
    P = params(**kw)
    Ff, G = dft_consts()
    kern = make_kernel(P)
    V = pltpu.VMEM
    scratch = [
        V((T, S, 128), bf16), V((T, S, 128), bf16), V((T, S, 128), bf16),
        V((KS, D), bf16), V((NC, D, 128), bf16), V((T, 128), bf16),
        V((T, D, 128), bf16), V((T, D, 128), bf16), V((T, F, 128), bf16), V((T, F, 128), bf16),
        V((1, 256, 128), bf16), V((2, 128, 128), bf16),
        V((KS, T, 8, 128), f32), V((T, 8, 128), f32),
        V((T, S + 8, 128), f32),
        V((NC, T, 128, 128), bf16),
        V((NC, 3, T, 128, 128), f32), V((NC, 3, T, 128, 128), f32), V((2, 2, T, 128, 128), f32),
        V((P["ZS"], T, 256, 128), bf16),
        V((P["XS"], T, 128, 128), f32), V((P["XS"], T, 128, 128), f32),
        V((T, S, 128), f32), V((T, S, 128), f32),
        V((P["RS"], T, 128, 128), bf16),
        V((T, S + 16, 128), f32),
        V((P["RS"], T, 128, 128), bf16),
        V((T, S, 128), f32),
        V((NC, T, 128, 128), bf16),
        V((P["YS"], NF, 128, 128), bf16),
        V((T, S, 128), bf16),
        pltpu.SemaphoreType.DMA((P["ngroups"],)), pltpu.SemaphoreType.DMA((1,)),
    ]

    def fn(A_q, A_k, A_v, A_shift_k, A_ssm_k, A_ssm_D, B_x, B_w1, B_w2, B_w3, B_w4):
        out = pl.pallas_call(
            kern,
            out_shape=jax.ShapeDtypeStruct((S, D), bf16),
            in_specs=[pl.BlockSpec(memory_space=pl.ANY)] * 12,
            out_specs=pl.BlockSpec(memory_space=pl.ANY),
            scratch_shapes=scratch,
            compiler_params=pltpu.CompilerParams(vmem_limit_bytes=120 * 1024 * 1024, flags=fl or None),
        )(A_q.reshape(S, D), A_k.reshape(S, D), A_v.reshape(S, D), A_shift_k.T, A_ssm_k, A_ssm_D.reshape(T, 128),
          B_w1, B_w2, B_w3.T, B_w4, jnp.asarray(Ff, bf16), jnp.asarray(G, bf16))
        return out.reshape(1, S, D)
    return fn


@jax.jit
def pallas_sequential_preLN__ssm_conv_h3__mixer_s_mlp__prompt_kernel(
    A_q: jax.Array,
    A_k: jax.Array,
    A_v: jax.Array,
    A_shift_k: jax.Array,
    A_ssm_k: jax.Array,
    A_ssm_D: jax.Array,
    B_x: jax.Array,
    B_w1: jax.Array,
    B_w2: jax.Array,
    B_w3: jax.Array,
    B_w4: jax.Array,
):
    return get_fn(rho="0.45", flags="XLA_TPU_RESCHEDULE_DMA_DONES", dma_groups="0-0|w1|1-1|2-2|3-3|w2|4-5|w3|6-7|w4|8-10|11-15", dma_times="2850,4600,6000,7400,8800,10500,13400,18000,20900,25600,30000,40000", ahead="3")(A_q, A_k, A_v, A_shift_k, A_ssm_k, A_ssm_D, B_x, B_w1, B_w2, B_w3, B_w4)
```
